```python
import jax
import jax.numpy as jnp

def _softmax(x, axis=-1):
    return jax.nn.softmax(x, axis=axis)
def _gelu(x):
    return jax.nn.gelu(x, approximate=True)
def _silu(x):
    return jax.nn.silu(x)
def _sigmoid(x):
    return jax.nn.sigmoid(x)
def _layernorm(x, axis=-1, eps=1e-5):
    m = jnp.mean(x, axis=axis, keepdims=True)
    v = jnp.var(x, axis=axis, keepdims=True)
    return (x - m) / jnp.sqrt(v + eps)
def _scatter_add(tgt, idx, src, axis=0):
    return tgt.at[idx].add(src)
def _segment_sum(src, seg, n):
    return jax.ops.segment_sum(src, seg, n)
class _Rng:
    def __init__(self, key):
        self._k = key
    def _next(self):
        self._k, sub = jax.random.split(self._k)
        return sub
    def normal(self, shape):
        return jax.random.normal(self._next(), shape, dtype=jnp.bfloat16)
    def randint(self, lo, hi, shape):
        return jax.random.randint(self._next(), shape, lo, hi, dtype=jnp.int32)
    def uniform(self, shape, lo=0.0, hi=1.0):
        return jax.random.uniform(self._next(), shape, jnp.bfloat16, lo, hi)
    def permutation(self, n):
        return jax.random.permutation(self._next(), n)


kernel_name = 'interleave_layers__linear_kernel_hedgehog__sliding_local_dilated__prompt'

def setup_inputs():
    _rng = _Rng(jax.random.key(int.from_bytes(__import__("os").urandom(4), "little")))
    _w = (lambda a: (lambda t: t.astype(jnp.bfloat16) if jnp.issubdtype(t.dtype, jnp.floating) else t)(jnp.asarray(a)))
    def _A_setup():
        B, S, D, H = 1, 2048, 1024, 32
        Dh = D // H
        return {
            "x": _w((lambda *s: _rng.normal(s) * 0.05)(B, S, D)),
            "wqkv": _w((lambda *s: _rng.normal(s) * 0.05)(D, 3 * D)),
            "w_phi": _w((lambda *s: _rng.normal(s) * 0.05)(H, Dh, Dh) * (Dh ** -0.5)),
            "wo": _w((lambda *s: _rng.normal(s) * 0.05)(D, D)),
        }
    _A_in = _A_setup()

    def _B_setup():
        B, S, D = 1, 2048, 1024
        return {
            "x": _w((lambda *s: _rng.normal(s) * 0.05)(B, S, D)),
            "wqkv": _w((lambda *s: _rng.normal(s) * 0.05)(D, 3 * D)),
            "wo": _w((lambda *s: _rng.normal(s) * 0.05)(D, D)),
        }
    _B_in = _B_setup()

    return {
        "A_x": _A_in["x"],
        "A_wqkv": _A_in["wqkv"],
        "A_w_phi": _A_in["w_phi"],
        "A_wo": _A_in["wo"],
        "B_x": _B_in["x"],
        "B_wqkv": _B_in["wqkv"],
        "B_wo": _B_in["wo"],
    }

def reference(A_x, A_wqkv, A_w_phi, A_wo, B_x, B_wqkv, B_wo):
    def _A_ref(x, wqkv, w_phi, wo):
        B, S, D = x.shape
        H = 32; Dh = D // H
        qkv = (lambda x, *d: x.transpose(*d))((x @ wqkv).reshape(B, S, 3, H, Dh), 2, 0, 3, 1, 4)
        q, k, v = qkv[0], qkv[1], qkv[2]
        pq = jnp.einsum("bhsd,hdf->bhsf", q, w_phi)
        pk = jnp.einsum("bhsd,hdf->bhsf", k, w_phi)
        phi_q = jnp.concatenate([_softmax(pq, axis=-1), _softmax(-pq, axis=-1)], axis=-1)
        phi_k = jnp.concatenate([_softmax(pk, axis=-1), _softmax(-pk, axis=-1)], axis=-1)
        kv = jnp.einsum("bhsf,bhsd->bhfd", phi_k, v)
        z  = jnp.einsum("bhsf->bhf", phi_k)
        num = jnp.einsum("bhqf,bhfd->bhqd", phi_q, kv)
        den = jnp.einsum("bhqf,bhf->bhq", phi_q, z)[..., None] + 1e-6
        o = num / den
        return (lambda x, *d: x.transpose(*d))(o, 0, 2, 1, 3).reshape(B, S, D) @ wo

    def _B_ref(x, wqkv, wo):
        B, S, D = x.shape
        H = 32; Dh = D // H
        W, dil = 8, 2
        qkv = (lambda x, *d: x.transpose(*d))((x @ wqkv).reshape(B, S, 3, H, Dh), 2, 0, 3, 1, 4)
        q, k, v = qkv[0], qkv[1], qkv[2]
        scale = Dh ** -0.5
        pos = jnp.arange(S)
        off = jnp.arange(W) * dil
        idx = pos[:, None] - off[None, :]
        mask = idx >= 0
        idx_c = jnp.where(mask, idx, 0).reshape(-1)
        kg = k[:, :, idx_c, :].reshape(B, H, S, W, Dh)
        vg = v[:, :, idx_c, :].reshape(B, H, S, W, Dh)
        logits = jnp.einsum("bhsd,bhswd->bhsw", q, kg) * scale
        logits = jnp.where(mask[None, None, :, :], logits, -1e9)
        attn = _softmax(logits, axis=-1)
        o = jnp.einsum("bhsw,bhswd->bhsd", attn, vg)
        return (lambda x, *d: x.transpose(*d))(o, 0, 2, 1, 3).reshape(B, S, D) @ wo

    x = A_x
    x = x + _A_ref(_layernorm(x, axis=-1), A_wqkv, A_w_phi, A_wo)
    x = x + _B_ref(_layernorm(x, axis=-1), B_wqkv, B_wo)
    x = x + _A_ref(_layernorm(x, axis=-1), A_wqkv, A_w_phi, A_wo)
    x = x + _B_ref(_layernorm(x, axis=-1), B_wqkv, B_wo)
    return x
```

```python
import functools
import math

import jax
import jax.numpy as jnp
import numpy as np
from jax.experimental import pallas as pl
from jax.experimental.pallas import tpu as pltpu

f32 = jnp.float32
bf16 = jnp.bfloat16

S = 2048
D = 1024
H = 32
DH = 32
C = 256
NC = S // C
LOG2E = math.log2(math.e)
HALO = 16


def _nt(a, b):
    return jax.lax.dot_general(a, b, (((1,), (1,)), ((), ())), preferred_element_type=f32)


def _nn(a, b):
    return jnp.dot(a, b, preferred_element_type=f32)


def _rcp(d):
    r = pl.reciprocal(d, approx=True)
    return r * (2.0 - d * r)


def _layernorm(x):
    m = jnp.mean(x, axis=-1, keepdims=True)
    xc = x - m
    v = jnp.mean(xc * xc, axis=-1, keepdims=True)
    return (xc * jax.lax.rsqrt(v + 1e-5)).astype(bf16)


def _feature_map(p):
    t = p.shape[1]
    p3 = p.reshape(H, DH, t)
    mx = jnp.max(p3, axis=1, keepdims=True)
    mn = jnp.min(p3, axis=1, keepdims=True)
    ep = jnp.exp2(p3 - mx)
    en = jnp.exp2(mn - p3)
    rp = _rcp(jnp.sum(ep, axis=1, keepdims=True))
    rn = _rcp(jnp.sum(en, axis=1, keepdims=True))
    phi = jnp.concatenate([ep * rp, en * rn], axis=1)
    return phi.reshape(2 * D, t)


def _permute_rows(w):
    n = w.shape[1]
    return jnp.swapaxes(w.reshape(H, DH, n), 0, 1).reshape(D, n)


def _kernel(x_hbm, wA_hbm, wphi_ref, woA_hbm, wB_hbm, woB_hbm, out_hbm,
            xs, wA, wqkT, woA, wB, woBs, wBT, woB, phiq, xres, kvacc, zacc, kvz,
            kscr, vscr, ostage, sem_in, sem_out):
    def cp_x(c):
        return pltpu.make_async_copy(x_hbm.at[pl.ds(c * C, C), :], xs.at[pl.ds(c * C, C), :], sem_in.at[c])

    def cp_wA(i):
        return pltpu.make_async_copy(wA_hbm.at[:, pl.ds(i * D, D)], wA.at[:, pl.ds(i * D, D)], sem_in.at[NC + i])

    def cp_wB(i):
        return pltpu.make_async_copy(wB_hbm.at[:, pl.ds(i * D, D)], wB.at[:, pl.ds(i * D, D)], sem_in.at[NC + 3 + i])

    cp_woA = pltpu.make_async_copy(woA_hbm, woA, sem_in.at[NC + 6])
    cp_woB = pltpu.make_async_copy(woB_hbm, woBs, sem_in.at[NC + 7])

    cp_x(0).start()
    cp_wA(1).start()
    cp_x(1).start()
    cp_wA(2).start()
    cp_wA(0).start()
    for c in range(2, NC):
        cp_x(c).start()
    for i in range(3):
        cp_wB(i).start()
    cp_woB.start()
    cp_woA.start()

    def bd_phi_t(g):
        wp = wphi_ref[g * 128:(g + 1) * 128, :].astype(f32)
        wt = jnp.concatenate([wp] * 4, axis=1)
        r = jax.lax.broadcasted_iota(jnp.int32, (128, 128), 0) // DH
        cc = jax.lax.broadcasted_iota(jnp.int32, (128, 128), 1) // DH
        return jnp.where(r == cc, wt, 0.0).T.astype(bf16)

    def fold(i):
        dst = 0 if i == 1 else D
        for g in range(8):
            r = _nt(bd[g], wA[:, i * D + g * 128: i * D + (g + 1) * 128])
            wqkT[dst + g * 128: dst + (g + 1) * 128, :] = (r * LOG2E).astype(bf16)

    def prep_wB(i, part, nparts):
        k0 = part * (D // nparts)
        w = wB[k0:k0 + D // nparts, i * D:(i + 1) * D].astype(f32).T
        wBT[i * D:(i + 1) * D, k0:k0 + D // nparts] = _permute_rows(w).astype(bf16)

    def prep_woB(part, nparts):
        k0 = part * (D // nparts)
        w = woBs[:, k0:k0 + D // nparts].astype(f32)
        woB[:, k0:k0 + D // nparts] = _permute_rows(w).astype(bf16)

    def ln_x0(c):
        return _layernorm(xs[c * C:(c + 1) * C, :].astype(f32))

    def m_pk(xn):
        return _nt(wqkT[0:D, :], xn)

    def m_pq(xn):
        return _nt(wqkT[D:2 * D, :], xn)

    def m_v(xn):
        return _nn(xn, wA[:, 2 * D:3 * D]).astype(bf16)

    def v_phik(pk, first):
        phi = _feature_map(pk)
        zs = phi[:, 0:128]
        for t in range(1, C // 128):
            zs = zs + phi[:, t * 128:(t + 1) * 128]
        if first:
            zacc[...] = zs
        else:
            zacc[...] += zs
        return phi.astype(bf16)

    def v_phiq(pq, c):
        phiq[:, c * C:(c + 1) * C] = _feature_map(pq).astype(bf16)

    def m_kv(phik, v, first):
        for g in range(8):
            r = _nn(phik[g * 256:(g + 1) * 256, :], v[:, g * 128:(g + 1) * 128])
            if first:
                kvacc[g] = r
            else:
                kvacc[g] += r

    def finalize_kv():
        rr = jax.lax.broadcasted_iota(jnp.int32, (256, 128), 0) // 64
        cc = jax.lax.broadcasted_iota(jnp.int32, (256, 128), 1)
        for g in range(8):
            kv = jnp.where(rr == cc // DH, kvacc[g], 0.0)
            z = jnp.sum(zacc[g * 256:(g + 1) * 256, :], axis=1, keepdims=True)
            zm = jnp.where(rr == cc // 8, z, 0.0)
            kvz[g, 0:128, :] = kv.T.astype(bf16)
            kvz[g, 128:160, :] = zm.T[0:32, :].astype(bf16)

    def m_num(c):
        return [_nn(kvz[g], phiq[g * 256:(g + 1) * 256, c * C:(c + 1) * C]) for g in range(8)]

    def v_o(nums):
        outs = []
        for g in range(8):
            num = nums[g][0:128, :].reshape(4, DH, C)
            den = nums[g][128:160, :].reshape(4, 8, C) + 1e-6
            r = _rcp(den)
            r = jnp.concatenate([r] * 4, axis=1)
            outs.append((num * r).reshape(128, C).astype(bf16))
        ot = jnp.concatenate(outs, axis=0)
        return ot.T

    def m_woA(o):
        return _nn(o, woA[...])

    def m_woB(o):
        return _nn(o, woB[...])

    def m_kB(xn, slot):
        k = _nt(xn, wBT[D:2 * D, :])
        for j in range(8):
            kscr[j, HALO + slot * C: HALO + (slot + 1) * C, :] = k[:, j * 128:(j + 1) * 128]

    def m_vB(xn, slot):
        v = _nt(xn, wBT[2 * D:3 * D, :])
        for j in range(8):
            vscr[j, HALO + slot * C: HALO + (slot + 1) * C, :] = v[:, j * 128:(j + 1) * 128]

    def m_qB(xn):
        return _nt(xn, wBT[0:D, :]) * (DH ** -0.5 * LOG2E)

    def v_attn(q, slot, c):
        base = HALO + slot * C
        lg = []
        row = jax.lax.broadcasted_iota(jnp.int32, (C, 128), 0)
        for w in range(8):
            acc = None
            for j in range(8):
                t = q[:, j * 128:(j + 1) * 128] * kscr[j, base - 2 * w: base - 2 * w + C, :]
                acc = t if acc is None else acc + t
            acc = acc + pltpu.roll(acc, 64, 1)
            acc = acc + pltpu.roll(acc, 32, 1)
            if c == 0 and w > 0:
                acc = jnp.where(row >= 2 * w, acc, -1e9 * LOG2E)
            lg.append(acc)
        m = lg[0]
        for w in range(1, 8):
            m = jnp.maximum(m, lg[w])
        e = [jnp.exp2(l - m) for l in lg]
        s = e[0]
        for w in range(1, 8):
            s = s + e[w]
        r = _rcp(s)
        a = [x * r for x in e]
        outs = []
        for j in range(8):
            acc = None
            for w in range(8):
                t = a[w] * vscr[j, base - 2 * w: base - 2 * w + C, :]
                acc = t if acc is None else acc + t
            outs.append(acc.astype(bf16))
        return jnp.concatenate(outs, axis=1)

    def halo_init():
        kscr[:, 0:HALO, :] = jnp.zeros((8, HALO, 128), f32)
        vscr[:, 0:HALO, :] = jnp.zeros((8, HALO, 128), f32)

    def halo_copy():
        kscr[:, 0:HALO, :] = kscr[:, 2 * C: 2 * C + HALO, :]
        vscr[:, 0:HALO, :] = vscr[:, 2 * C: 2 * C + HALO, :]

    bd = [bd_phi_t(g) for g in range(8)]
    cp_x(0).wait()
    xn = {}
    xn[0] = ln_x0(0)
    cp_wA(1).wait()
    fold(1)
    cp_x(1).wait()
    xn[1] = ln_x0(1)

    def a_part_pair(a, b, xa, xb, first, last, between=None):
        pk_a = m_pk(xa)
        if between: between(0)
        v_a = m_v(xa)
        phik_a = v_phik(pk_a, first)
        pk_b = m_pk(xb)
        v_b = m_v(xb)
        phik_b = v_phik(pk_b, False)
        pq_a = m_pq(xa)
        m_kv(phik_a, v_a, first)
        m_kv(phik_b, v_b, False)
        if last:
            finalize_kv()
        v_phiq(pq_a, a)
        pq_b = m_pq(xb)
        v_phiq(pq_b, b)

    for it in range(NC // 2):
        a, b = 2 * it, 2 * it + 1
        if it == 0:
            def between(k):
                cp_wA(2).wait()
            pk_a = m_pk(xn[0])
            cp_wA(2).wait()
            v_a = m_v(xn[0])
            phik_a = v_phik(pk_a, True)
            pk_b = m_pk(xn[1])
            v_b = m_v(xn[1])
            phik_b = v_phik(pk_b, False)
            cp_wA(0).wait()
            fold(0)
            for c in (2, 3):
                cp_x(c).wait()
                xn[c] = ln_x0(c)
            pq_a = m_pq(xn[0])
            m_kv(phik_a, v_a, True)
            m_kv(phik_b, v_b, False)
            v_phiq(pq_a, 0)
            pq_b = m_pq(xn[1])
            v_phiq(pq_b, 1)
        else:
            if it == 1:
                for i in range(3):
                    cp_wB(i).wait()
                cp_woB.wait()
            last = it == NC // 2 - 1
            pk_a = m_pk(xn[a])
            prep_wB(0, it - 1, 3) if False else None
            v_a = m_v(xn[a])
            phik_a = v_phik(pk_a, False)
            pk_b = m_pk(xn[b])
            v_b = m_v(xn[b])
            phik_b = v_phik(pk_b, False)
            if not last:
                for c in (a + 2, b + 2):
                    cp_x(c).wait()
                    xn[c] = ln_x0(c)
            if it == 1:
                prep_wB(1, 0, 1)
            elif it == 2:
                prep_wB(2, 0, 1)
            else:
                prep_wB(0, 0, 1)
                prep_woB(0, 1)
            pq_a = m_pq(xn[a])
            m_kv(phik_a, v_a, False)
            m_kv(phik_b, v_b, False)
            if last:
                finalize_kv()
            v_phiq(pq_a, a)
            pq_b = m_pq(xn[b])
            v_phiq(pq_b, b)
    cp_woA.wait()

    def b_pair(it, final):
        a, b = 2 * it, 2 * it + 1
        if it == 0:
            halo_init()
        else:
            halo_copy()
        nums_a = m_num(a)
        nums_b = m_num(b)
        o_a = v_o(nums_a)
        o_b = v_o(nums_b)
        if final:
            xa = xres[a * C:(a + 1) * C, :]
            xb = xres[b * C:(b + 1) * C, :]
        else:
            xa = xs[a * C:(a + 1) * C, :].astype(f32)
            xb = xs[b * C:(b + 1) * C, :].astype(f32)
        x1a = xa + m_woA(o_a)
        x1b = xb + m_woA(o_b)
        xna = _layernorm(x1a)
        xnb = _layernorm(x1b)
        m_kB(xna, 0)
        m_vB(xna, 0)
        q_a = m_qB(xna)
        m_kB(xnb, 1)
        m_vB(xnb, 1)
        q_b = m_qB(xnb)
        at_a = v_attn(q_a, 0, a)
        at_b = v_attn(q_b, 1, b)
        x2a = x1a + m_woB(at_a)
        x2b = x1b + m_woB(at_b)
        return x2a, x2b

    for it in range(NC // 2):
        a, b = 2 * it, 2 * it + 1
        x2a, x2b = b_pair(it, False)
        xres[a * C:(a + 1) * C, :] = x2a
        xres[b * C:(b + 1) * C, :] = x2b
        xna = _layernorm(x2a)
        xnb = _layernorm(x2b)
        pk_a = m_pk(xna)
        v_a = m_v(xna)
        phik_a = v_phik(pk_a, it == 0)
        pk_b = m_pk(xnb)
        v_b = m_v(xnb)
        phik_b = v_phik(pk_b, False)
        pq_a = m_pq(xna)
        m_kv(phik_a, v_a, it == 0)
        m_kv(phik_b, v_b, False)
        pq_b = m_pq(xnb)
        v_phiq(pq_a, a)
        v_phiq(pq_b, b)
    finalize_kv()

    def cp_out(it):
        slot = it % 2
        return pltpu.make_async_copy(ostage.at[slot], out_hbm.at[pl.ds(it * 2 * C, 2 * C), :], sem_out.at[slot])

    for it in range(NC // 2):
        x2a, x2b = b_pair(it, True)
        if it >= 2:
            cp_out(it - 2).wait()
        ostage[it % 2, 0:C, :] = x2a.astype(bf16)
        ostage[it % 2, C:2 * C, :] = x2b.astype(bf16)
        cp_out(it).start()
    cp_out(NC // 2 - 2).wait()
    cp_out(NC // 2 - 1).wait()


@jax.jit
def pallas_interleave_layers__linear_kernel_hedgehog__sliding_local_dilated__prompt_kernel(
    A_x, A_wqkv, A_w_phi, A_wo, B_x, B_wqkv, B_wo,
):
    del B_x
    x = A_x.reshape(S, D)
    wphi = A_w_phi.reshape(H * DH, DH)
    any_spec = pl.BlockSpec(memory_space=pl.ANY)
    out = pl.pallas_call(
        _kernel,
        out_shape=jax.ShapeDtypeStruct((S, D), bf16),
        in_specs=[any_spec, any_spec, pl.BlockSpec(memory_space=pltpu.VMEM), any_spec, any_spec, any_spec],
        out_specs=any_spec,
        scratch_shapes=[
            pltpu.VMEM((S, D), bf16),
            pltpu.VMEM((D, 3 * D), bf16),
            pltpu.VMEM((2 * D, D), bf16),
            pltpu.VMEM((D, D), bf16),
            pltpu.VMEM((D, 3 * D), bf16),
            pltpu.VMEM((D, D), bf16),
            pltpu.VMEM((3 * D, D), bf16),
            pltpu.VMEM((D, D), bf16),
            pltpu.VMEM((2 * D, S), bf16),
            pltpu.VMEM((S, D), f32),
            pltpu.VMEM((8, 256, 128), f32),
            pltpu.VMEM((2 * D, 128), f32),
            pltpu.VMEM((8, 160, 256), bf16),
            pltpu.VMEM((8, HALO + 2 * C, 128), f32),
            pltpu.VMEM((8, HALO + 2 * C, 128), f32),
            pltpu.VMEM((2, 2 * C, D), bf16),
            pltpu.SemaphoreType.DMA((NC + 8,)),
            pltpu.SemaphoreType.DMA((2,)),
        ],
        compiler_params=pltpu.CompilerParams(vmem_limit_bytes=120 * 1024 * 1024),
        name="hedgehog_sliding_fused",
    )(x, A_wqkv, wphi, A_wo, B_wqkv, B_wo)
    return out.reshape(1, S, D)
```

```python
import math
import os

import jax
import jax.numpy as jnp
import numpy as np
from jax.experimental import pallas as pl
from jax.experimental.pallas import tpu as pltpu

f32 = jnp.float32
bf16 = jnp.bfloat16
u32 = jnp.uint32

S = 2048
D = 1024
H = 32
DH = 32
C = 256
NC = S // C
LOG2E = math.log2(math.e)
HALO = 16
RB = 16
PH = os.environ.get('PH', '123')


def _nt(a, b):
    return jax.lax.dot_general(a, b, (((1,), (1,)), ((), ())), preferred_element_type=f32)


def _nn(a, b):
    return jnp.dot(a, b, preferred_element_type=f32)


def _pk(x):
    return pltpu.bitcast(x, u32)


def _upk(x):
    return pltpu.bitcast(x, bf16)


def _rcp(d):
    r = pl.reciprocal(d, approx=True)
    return r * (2.0 - d * r)


def _layernorm(x):
    m = jnp.mean(x, axis=-1, keepdims=True)
    xc = x - m
    v = jnp.mean(xc * xc, axis=-1, keepdims=True)
    return (xc * jax.lax.rsqrt(v + 1e-5)).astype(bf16)


def _feature_map(p):
    t = p.shape[1]
    p3 = p.reshape(H, DH, t)
    mx = jnp.max(p3, axis=1, keepdims=True)
    mn = jnp.min(p3, axis=1, keepdims=True)
    ep = jnp.exp2(p3 - mx)
    en = jnp.exp2(mn - p3)
    rp = _rcp(jnp.sum(ep, axis=1, keepdims=True))
    rn = _rcp(jnp.sum(en, axis=1, keepdims=True))
    phi = jnp.concatenate([ep * rp, en * rn], axis=1)
    return phi.reshape(2 * D, t)


def _kernel(x_hbm, wA_hbm, wphi_ref, woA_hbm, wB_hbm, woB_hbm, out_hbm,
            xs, wA, wAT, woAs, woA, wB, woBs, wBT, woB, perm, phiq, xres, kvacc, kvz,
            kscr, vscr, t0, t1, ostage, sem_in, sem_out):
    def cp_x(c):
        return pltpu.make_async_copy(x_hbm.at[pl.ds(c * C, C), :], xs.at[pl.ds(c * C, C), :], sem_in.at[c])

    def cp_wA(i):
        return pltpu.make_async_copy(wA_hbm.at[:, pl.ds(i * D, D)], wA.at[:, pl.ds(i * D, D)], sem_in.at[NC + i])

    cp_wB = pltpu.make_async_copy(wB_hbm, wB, sem_in.at[NC + 3])
    cp_woA = pltpu.make_async_copy(woA_hbm, woAs, sem_in.at[NC + 4])
    cp_woB = pltpu.make_async_copy(woB_hbm, woBs, sem_in.at[NC + 5])

    def bd_phi_t(g):
        wp = wphi_ref[g * 128:(g + 1) * 128, :].astype(f32)
        wt = jnp.concatenate([wp] * 4, axis=1)
        r = jax.lax.broadcasted_iota(jnp.int32, (128, 128), 0) // DH
        cc = jax.lax.broadcasted_iota(jnp.int32, (128, 128), 1) // DH
        return jnp.where(r == cc, wt, 0.0).T.astype(bf16)

    def fold(i):
        dst = 0 if i == 1 else D
        for g in range(8):
            r = _nt(bd[g], wA[:, i * D + g * 128: i * D + (g + 1) * 128])
            wAT[dst + g * 64: dst + (g + 1) * 64, :] = _pk((r * LOG2E).astype(bf16))

    def prep_wvT():
        wAT[512:1024, :] = _pk(wA[:, 2 * D:3 * D].T)

    def permute_store(val, dst_ref, row0, col0):
        for h in range(H):
            perm[pl.ds(h, DH, stride=DH + 1), :] = val[h * DH:(h + 1) * DH, :]
        rows = [perm[(DH + 1) * r:(DH + 1) * r + DH, :] for r in range(DH)]
        dst_ref[row0:row0 + 512, col0:col0 + 128] = _pk(jnp.concatenate(rows, axis=0).astype(bf16))

    def prep_wB(i, s):
        w = wB[s * 128:(s + 1) * 128, i * D:(i + 1) * D].astype(f32).T
        permute_store(w, wBT, i * 512, s * 128)

    def prep_woB(s):
        permute_store(woBs[:, s * 128:(s + 1) * 128].astype(f32), woB, 0, s * 128)

    def prep_woA():
        woA[...] = _pk(woAs[...])

    val = {}

    def ln_x0(c):
        val['xn', c] = _layernorm(xs[c * C:(c + 1) * C, :].astype(f32))

    def m_pk(c):
        val['pk', c] = _nt(_upk(wAT[0:512, :]), val['xn', c])

    def m_vT(c):
        val['vT', c] = _nt(_upk(wAT[512:1024, :]), val['xn', c]).astype(bf16)

    def m_pq(c):
        val['pq', c] = _nt(_upk(wAT[1024:1536, :]), val['xn', c])

    def v_phik(c):
        val['phik', c] = _feature_map(val.pop(('pk', c))).astype(bf16)

    def v_phiq(c):
        phiq[:, c * C:(c + 1) * C] = _pk(_feature_map(val.pop(('pq', c))).astype(bf16))

    def m_kv(c):
        phik = val.pop(('phik', c))
        vt = val.pop(('vT', c))
        ones = jnp.ones((16, C), bf16)
        for hp in range(16):
            lhs = jnp.concatenate([vt[hp * 64:(hp + 1) * 64, :], ones], axis=0)
            r = _nt(lhs, phik[hp * 128:(hp + 1) * 128, :])
            if c == 0:
                kvacc[hp] = r
            else:
                kvacc[hp] += r

    def finalize_kv():
        row = jax.lax.broadcasted_iota(jnp.int32, (80, 128), 0)
        head = jnp.where(row < 64, row // DH, (row - 64) // 8)
        keep = head == jax.lax.broadcasted_iota(jnp.int32, (80, 128), 1) // 64
        for hp in range(16):
            kvz[hp] = _pk(jnp.where(keep, kvacc[hp], 0.0).astype(bf16))

    def m_num(c):
        val['num', c] = [_nn(_upk(kvz[hp]), _upk(phiq[hp * 64:(hp + 1) * 64, c * C:(c + 1) * C]))
                         for hp in range(16)]

    def v_o(c):
        nums = val.pop(('num', c))
        outs = []
        for hp in range(16):
            num = nums[hp][0:64, :].reshape(2, DH, C)
            den = nums[hp][64:80, :].reshape(2, 8, C) + 1e-6
            r = _rcp(den)
            r = jnp.concatenate([r] * 4, axis=1)
            outs.append((num * r).reshape(64, C).astype(bf16))
        val['o', c] = jnp.concatenate(outs, axis=0).T

    def m_woA(c, final):
        x = xres[c * C:(c + 1) * C, :] if final else xs[c * C:(c + 1) * C, :].astype(f32)
        val['x1', c] = x + _nn(val.pop(('o', c)), _upk(woA[...]))

    def v_ln1(c):
        val['xn1', c] = _layernorm(val['x1', c])

    def m_kB(c):
        k = _nt(val['xn1', c], _upk(wBT[512:1024, :]))
        for j in range(8):
            kscr[j, HALO + c * C: HALO + (c + 1) * C, :] = k[:, j * 128:(j + 1) * 128]

    def m_qB(c):
        t = t0 if c % 2 == 0 else t1
        q = _nt(val['xn1', c], _upk(wBT[0:512, :])) * (DH ** -0.5 * LOG2E)
        for j in range(8):
            t[j] = q[:, j * 128:(j + 1) * 128]

    def m_vB(c):
        v = _nt(val.pop(('xn1', c)), _upk(wBT[1024:1536, :]))
        for j in range(8):
            vscr[j, HALO + c * C: HALO + (c + 1) * C, :] = v[:, j * 128:(j + 1) * 128]

    def v_logits(c):
        t = t0 if c % 2 == 0 else t1
        base = HALO + c * C
        for r0 in range(0, C, RB):
            rr = r0
            row = jax.lax.broadcasted_iota(jnp.int32, (RB, 128), 0) + r0
            qs = [t[j, pl.ds(rr, RB), :] for j in range(8)]
            lg = []
            for w in range(8):
                acc = None
                for j in range(8):
                    p = qs[j] * kscr[j, base + r0 - 2 * w: base + r0 - 2 * w + RB, :]
                    acc = p if acc is None else acc + p
                acc = acc + pltpu.roll(acc, 64, 1)
                acc = acc + pltpu.roll(acc, 32, 1)
                if c == 0 and w > 0 and r0 < 16:
                    acc = jnp.where(row >= 2 * w, acc, -1e9 * LOG2E)
                lg.append(acc)
            m = lg[0]
            for w in range(1, 8):
                m = jnp.maximum(m, lg[w])
            e = [jnp.exp2(l - m) for l in lg]
            s = e[0]
            for w in range(1, 8):
                s = s + e[w]
            r = _rcp(s)
            for w in range(8):
                t[8 + w, r0:r0 + RB, :] = e[w] * r

    def v_pv(c):
        t = t0 if c % 2 == 0 else t1
        base = HALO + c * C
        for r0 in range(0, C, RB):
            rr = r0
            a = [t[8 + w, pl.ds(rr, RB), :] for w in range(8)]
            for j in range(8):
                acc = None
                for w in range(8):
                    p = a[w] * vscr[j, base + r0 - 2 * w: base + r0 - 2 * w + RB, :]
                    acc = p if acc is None else acc + p
                t[16 + j, r0 // 2:(r0 + RB) // 2, :] = pltpu.bitcast(acc.astype(bf16), f32)

    def m_woB(c):
        t = t0 if c % 2 == 0 else t1
        at = jnp.concatenate([_upk(t[16 + j, 0:C // 2, :]) for j in range(8)], axis=1)
        val['x2', c] = val.pop(('x1', c)) + _nn(at, _upk(woB[...]))

    def v_ln2(c):
        x2 = val.pop(('x2', c))
        xres[c * C:(c + 1) * C, :] = x2
        val['xn', c] = _layernorm(x2)

    def v_out(c):
        ostage[c * C:(c + 1) * C, :] = val.pop(('x2', c)).astype(bf16)
        pltpu.make_async_copy(ostage.at[pl.ds(c * C, C), :], out_hbm.at[pl.ds(c * C, C), :], sem_out.at[c]).start()

    cp_x(0).start()
    cp_wA(1).start()
    cp_x(1).start()
    cp_wA(2).start()
    cp_wA(0).start()
    kscr[:, 0:HALO, :] = jnp.zeros((8, HALO, 128), f32)
    vscr[:, 0:HALO, :] = jnp.zeros((8, HALO, 128), f32)
    bd = [bd_phi_t(g) for g in range(8)]
    cp_x(0).wait()
    cp_wA(1).wait()
    ln_x0(0)
    fold(1)

    if '1' in PH:
        m_pk(0)
        cp_x(1).wait()
        cp_wA(2).wait()
        for c in range(2, NC):
            cp_x(c).start()
        ln_x0(1)
        prep_wvT()
        m_pk(1)
        v_phik(0)
        m_vT(0)
        v_phik(1)
        m_vT(1)
        m_kv(0)
        m_kv(1)
        cp_wA(0).wait()
        cp_wB.start()
        cp_woB.start()
        cp_woA.start()
        fold(0)
        m_pq(0)
        for c in range(2, NC):
            cp_x(c).wait()
        v_phiq(0)
        for c in range(2, NC):
            ln_x0(c)
        m_pq(1)
        v_phiq(1)
        for c in range(2, NC):
            if c == 4:
                cp_wB.wait()
                cp_woB.wait()
                cp_woA.wait()
                prep_woA()
                for i in (1, 0, 2):
                    for s in range(8):
                        prep_wB(i, s)
                for s in range(8):
                    prep_woB(s)
            m_pk(c)
            v_phik(c)
            m_vT(c)
            if c < NC - 1:
                m_pq(c)
                v_phiq(c)
            m_kv(c)
        finalize_kv()

    def b_phase(final):
        m_num(0)
        m_num(1)
        m_pq(NC - 1)
        v_phiq(NC - 1)
        v_o(0)
        for t in range(-1, NC + 2):
            if 2 <= t + 2 < NC:
                m_num(t + 2)
            if 0 <= t + 2 < NC and t + 2 > 0:
                v_o(t + 2)
            if 0 <= t + 1 < NC:
                m_woA(t + 1, final)
                v_ln1(t + 1)
            if 0 <= t < NC:
                m_kB(t)
                m_qB(t)
                v_logits(t)
                m_vB(t)
                v_pv(t)
            if 0 <= t - 1 < NC:
                m_woB(t - 1)
                if final:
                    v_out(t - 1)
                else:
                    v_ln2(t - 1)
            if not final and 0 <= t - 2 < NC:
                c = t - 2
                m_pk(c)
                v_phik(c)
                m_vT(c)
                if c < NC - 1:
                    m_pq(c)
                    v_phiq(c)
                m_kv(c)
        if not final:
            finalize_kv()

    if '1' not in PH:
        val['xn', NC - 1] = val['xn', 0]
    if '2' in PH:
        b_phase(False)
    if '3' in PH:
        b_phase(True)
        for c in range(NC):
            pltpu.make_async_copy(ostage.at[pl.ds(c * C, C), :], out_hbm.at[pl.ds(c * C, C), :], sem_out.at[c]).wait()


@jax.jit
def pallas_interleave_layers__linear_kernel_hedgehog__sliding_local_dilated__prompt_kernel(
    A_x, A_wqkv, A_w_phi, A_wo, B_x, B_wqkv, B_wo,
):
    del B_x
    x = A_x.reshape(S, D)
    wphi = A_w_phi.reshape(H * DH, DH)
    any_spec = pl.BlockSpec(memory_space=pl.ANY)
    out = pl.pallas_call(
        _kernel,
        out_shape=jax.ShapeDtypeStruct((S, D), bf16),
        in_specs=[any_spec, any_spec,
                  pl.BlockSpec(memory_space=pltpu.VMEM), any_spec, any_spec, any_spec],
        out_specs=any_spec,
        scratch_shapes=[
            pltpu.VMEM((S, D), bf16),
            pltpu.VMEM((D, 3 * D), bf16),
            pltpu.VMEM((3 * D // 2, D), u32),
            pltpu.VMEM((D, D), bf16),
            pltpu.VMEM((D // 2, D), u32),
            pltpu.VMEM((D, 3 * D), bf16),
            pltpu.VMEM((D, D), bf16),
            pltpu.VMEM((3 * D // 2, D), u32),
            pltpu.VMEM((D // 2, D), u32),
            pltpu.VMEM((DH * (DH + 1), 128), f32),
            pltpu.VMEM((D, S), u32),
            pltpu.VMEM((S, D), f32),
            pltpu.VMEM((16, 80, 128), f32),
            pltpu.VMEM((16, 40, 128), u32),
            pltpu.VMEM((8, HALO + S, 128), f32),
            pltpu.VMEM((8, HALO + S, 128), f32),
            pltpu.VMEM((24, C, 128), f32),
            pltpu.VMEM((24, C, 128), f32),
            pltpu.VMEM((S, D), bf16),
            pltpu.SemaphoreType.DMA((NC + 6,)),
            pltpu.SemaphoreType.DMA((NC,)),
        ],
        compiler_params=pltpu.CompilerParams(vmem_limit_bytes=124 * 1024 * 1024),
        name="hedgehog_sliding_fused",
    )(x, A_wqkv, wphi, A_wo, B_wqkv, B_wo)
    return out.reshape(1, S, D)
```

```python
import math

import jax
import jax.numpy as jnp
import numpy as np
from jax.experimental import pallas as pl
from jax.experimental.pallas import tpu as pltpu

f32 = jnp.float32
bf16 = jnp.bfloat16
u32 = jnp.uint32

S = 2048
D = 1024
H = 32
DH = 32
C = 256
NC = S // C
LOG2E = math.log2(math.e)
HALO = 16
RB = 32


def _nt(a, b):
    return jax.lax.dot_general(a, b, (((1,), (1,)), ((), ())), preferred_element_type=f32)


def _nn(a, b):
    return jnp.dot(a, b, preferred_element_type=f32)


def _pk(x):
    return pltpu.bitcast(x, u32)


def _upk(x):
    return pltpu.bitcast(x, bf16)


def _rcp(d):
    r = pl.reciprocal(d, approx=True)
    return r * (2.0 - d * r)


def _layernorm(x):
    m = jnp.mean(x, axis=-1, keepdims=True)
    xc = x - m
    v = jnp.mean(xc * xc, axis=-1, keepdims=True)
    return (xc * jax.lax.rsqrt(v + 1e-5)).astype(bf16)


def _layernorm_ref(load):
    m = jnp.mean(load(), axis=-1, keepdims=True)
    xc = load() - m
    r = jax.lax.rsqrt(jnp.mean(xc * xc, axis=-1, keepdims=True) + 1e-5)
    return (load() * r - m * r).astype(bf16)


def _feature_map(p):
    t = p.shape[1]
    p3 = p.reshape(H, DH, t)
    mx = jnp.max(p3, axis=1, keepdims=True)
    mn = jnp.min(p3, axis=1, keepdims=True)
    ep = jnp.exp2(p3 - mx)
    en = jnp.exp2(mn - p3)
    rp = _rcp(jnp.sum(ep, axis=1, keepdims=True))
    rn = _rcp(jnp.sum(en, axis=1, keepdims=True))
    phi = jnp.concatenate([ep * rp, en * rn], axis=1)
    return phi.reshape(2 * D, t)


def _kernel(x_hbm, wA_hbm, wphi_hbm, woA_hbm, wB_hbm, woB_hbm, out_hbm,
            wphi_ref, x1s, xs, wA, wAT, woAs, woA, wB, woBs, wBT, woB, perm, phiq, xres, kvacc, kvz,
            kscr, vscr, t0, t1, ostage, sem_in, sem_out):
    def cp_x(c):
        return pltpu.make_async_copy(x_hbm.at[pl.ds(c * C, C), :], xs.at[pl.ds(c * C, C), :], sem_in.at[c])

    def cp_wA(i):
        return pltpu.make_async_copy(wA_hbm.at[:, pl.ds(i * D, D)], wA.at[pl.ds(0, D), pl.ds(i * D, D)], sem_in.at[NC + i])

    def cp_wB(i):
        return pltpu.make_async_copy(wB_hbm.at[:, pl.ds(i * D, D)], wB.at[pl.ds(0, D), pl.ds(i * D, D)], sem_in.at[NC + 6 + i])

    WK = [(0, 2), (2, 5), (5, 8)]

    def cp_wk(part):
        g0, g1 = WK[part]
        cols = pl.ds(D + g0 * 128, (g1 - g0) * 128)
        return pltpu.make_async_copy(wA_hbm.at[:, cols], wA.at[pl.ds(0, D), cols], sem_in.at[NC + 9 + part])

    cp_wphi = pltpu.make_async_copy(wphi_hbm, wphi_ref, sem_in.at[NC + 3])
    cp_woA = pltpu.make_async_copy(woA_hbm, woAs.at[pl.ds(0, D), :], sem_in.at[NC + 4])
    cp_woB = pltpu.make_async_copy(woB_hbm, woBs.at[pl.ds(0, D), :], sem_in.at[NC + 5])

    def bd_phi_t(g):
        wp = wphi_ref[g * 128:(g + 1) * 128, :].astype(f32)
        wt = jnp.concatenate([wp] * 4, axis=1)
        r = jax.lax.broadcasted_iota(jnp.int32, (128, 128), 0) // DH
        cc = jax.lax.broadcasted_iota(jnp.int32, (128, 128), 1) // DH
        return jnp.where(r == cc, wt, 0.0).T.astype(bf16)

    def fold(i, groups=range(8)):
        dst = 0 if i == 1 else D
        for g in groups:
            r = _nt(bd[g], wA[0:D, i * D + g * 128: i * D + (g + 1) * 128])
            wAT[dst + g * 64: dst + (g + 1) * 64, :] = _pk((r * LOG2E).astype(bf16))

    def prep_wvT():
        wAT[512:1024, :] = _pk(wA[0:D, 2 * D:3 * D].T)

    def permute_store(val, dst_ref, row0, col0):
        b = (col0 // 128) % perm.shape[0]
        for h in range(H):
            perm[b, pl.ds(h, DH, stride=DH + 1), :] = val[h * DH:(h + 1) * DH, :]
        rows = [perm[b, (DH + 1) * r:(DH + 1) * r + DH, :] for r in range(DH)]
        dst_ref[row0:row0 + 512, col0:col0 + 128] = _pk(jnp.concatenate(rows, axis=0).astype(bf16))

    def prep_wB(i, s):
        w = wB[s * 128:(s + 1) * 128, i * D:(i + 1) * D].astype(f32).T
        permute_store(w, wBT, i * 512, s * 128)

    def prep_woB(s):
        permute_store(woBs[0:D, s * 128:(s + 1) * 128].astype(f32), woB, 0, s * 128)

    def prep_woA():
        woA[...] = _pk(woAs[0:D, :])

    val = {}

    def ln_x0(c):
        val['xn', c] = _layernorm(xs[c * C:(c + 1) * C, :].astype(f32))

    def m_pk(c):
        val['pk', c] = _nt(_upk(wAT[0:512, :]), val['xn', c])

    def m_vT(c):
        val['vT', c] = _nt(_upk(wAT[512:1024, :]), val['xn', c]).astype(bf16)

    def m_pq(c):
        val['pq', c] = _nt(_upk(wAT[1024:1536, :]), val['xn', c])

    def v_phik(c):
        val['phik', c] = _feature_map(val.pop(('pk', c))).astype(bf16)

    def v_phiq(c):
        phiq[:, c * C:(c + 1) * C] = _pk(_feature_map(val.pop(('pq', c))).astype(bf16))

    def m_kv(c):
        phik = val.pop(('phik', c))
        vt = val.pop(('vT', c))
        ones = jnp.ones((16, C), bf16)
        for hp in range(16):
            lhs = jnp.concatenate([ones, vt[hp * 64:(hp + 1) * 64, :]], axis=0)
            r = _nt(lhs, phik[hp * 128:(hp + 1) * 128, :])
            if c == 0:
                kvacc[hp] = r
            else:
                kvacc[hp] += r

    def finalize_kv():
        row = jax.lax.broadcasted_iota(jnp.int32, (80, 128), 0)
        head = jnp.where(row < 16, row // 8, (row - 16) // DH)
        keep = head == jax.lax.broadcasted_iota(jnp.int32, (80, 128), 1) // 64
        for hp in range(16):
            kvz[hp] = _pk(jnp.where(keep, kvacc[hp], 0.0).astype(bf16))

    def m_num(c):
        val['num', c] = [_nn(_upk(kvz[hp]), _upk(phiq[hp * 64:(hp + 1) * 64, c * C:(c + 1) * C]))
                         for hp in range(16)]

    def v_o(c):
        nums = val.pop(('num', c))
        outs = []
        for hp in range(16):
            num = nums[hp][16:80, :].reshape(2, DH, C)
            den = nums[hp][0:16, :].reshape(2, 8, C) + 1e-6
            r = _rcp(den)
            r = jnp.concatenate([r] * 4, axis=1)
            outs.append((num * r).reshape(64, C).astype(bf16))
        val['o', c] = jnp.concatenate(outs, axis=0).T

    def m_woA(c, final):
        x = xres[c * C:(c + 1) * C, :] if final else xs[c * C:(c + 1) * C, :].astype(f32)
        x1s[c % 3] = x + _nn(val.pop(('o', c)), _upk(woA[...]))

    def v_ln1(c):
        val['xn1', c] = _layernorm_ref(lambda: x1s[c % 3])

    def m_kB(c):
        k = _nt(val['xn1', c], _upk(wBT[512:1024, :]))
        for j in range(8):
            kscr[j, HALO + c * C: HALO + (c + 1) * C, :] = k[:, j * 128:(j + 1) * 128]

    def m_qB(c):
        t = t0 if c % 2 == 0 else t1
        q = _nt(val['xn1', c], _upk(wBT[0:512, :])) * (DH ** -0.5 * LOG2E)
        for j in range(8):
            t[j] = q[:, j * 128:(j + 1) * 128]

    def m_vB(c):
        v = _nt(val.pop(('xn1', c)), _upk(wBT[1024:1536, :]))
        for j in range(8):
            vscr[j, HALO + c * C: HALO + (c + 1) * C, :] = v[:, j * 128:(j + 1) * 128]

    def v_logits(c):
        t = t0 if c % 2 == 0 else t1
        base = HALO + c * C
        for r0 in range(0, C, RB):
            rr = r0
            row = jax.lax.broadcasted_iota(jnp.int32, (RB, 128), 0) + r0
            qs = [t[j, pl.ds(rr, RB), :] for j in range(8)]
            lg = []
            for w in range(8):
                acc = None
                for j in range(8):
                    p = qs[j] * kscr[j, base + r0 - 2 * w: base + r0 - 2 * w + RB, :]
                    acc = p if acc is None else acc + p
                acc = (acc + pltpu.roll(acc, 64, 1)) + (pltpu.roll(acc, 32, 1) + pltpu.roll(acc, 96, 1))
                if c == 0 and w > 0 and r0 < 16:
                    acc = jnp.where(row >= 2 * w, acc, -1e9 * LOG2E)
                lg.append(acc)
            m = lg[0]
            for w in range(1, 8):
                m = jnp.maximum(m, lg[w])
            e = [jnp.exp2(l - m) for l in lg]
            s = e[0]
            for w in range(1, 8):
                s = s + e[w]
            r = _rcp(s)
            for w in range(8):
                t[8 + w, r0:r0 + RB, :] = e[w] * r

    def v_pv(c):
        t = t0 if c % 2 == 0 else t1
        base = HALO + c * C
        for r0 in range(0, C, RB):
            rr = r0
            a = [t[8 + w, pl.ds(rr, RB), :] for w in range(8)]
            for j in range(8):
                acc = None
                for w in range(8):
                    p = a[w] * vscr[j, base + r0 - 2 * w: base + r0 - 2 * w + RB, :]
                    acc = p if acc is None else acc + p
                t[16 + j, r0 // 2:(r0 + RB) // 2, :] = pltpu.bitcast(acc.astype(bf16), f32)

    def m_woB(c, final):
        t = t0 if c % 2 == 0 else t1
        at = jnp.concatenate([_upk(t[16 + j, 0:C // 2, :]) for j in range(8)], axis=1)
        x2 = x1s[c % 3] + _nn(at, _upk(woB[...]))
        if final:
            val['x2', c] = x2
        else:
            xres[c * C:(c + 1) * C, :] = x2

    def v_ln2(c):
        val['xn', c] = _layernorm_ref(lambda: xres[c * C:(c + 1) * C, :])

    def v_out(c):
        ostage[c * C:(c + 1) * C, :] = val.pop(('x2', c)).astype(bf16)
        pltpu.make_async_copy(ostage.at[pl.ds(c * C, C), :], out_hbm.at[pl.ds(c * C, C), :], sem_out.at[c]).start()

    cp_wphi.start()
    cp_x(0).start()
    cp_wk(0).start()
    cp_wk(1).start()
    kscr[:, 0:HALO, :] = jnp.zeros((8, HALO, 128), f32)
    vscr[:, 0:HALO, :] = jnp.zeros((8, HALO, 128), f32)
    cp_wphi.wait()
    cp_x(0).wait()
    bd = [bd_phi_t(g) for g in range(8)]
    ln_x0(0)
    pk0 = []
    for part in range(3):
        g0, g1 = WK[part]
        cp_wk(part).wait()
        if part == 0:
            cp_wk(2).start()
            cp_x(1).start()
        if part == 1:
            cp_x(1).wait()
            cp_wA(2).start()
        if part == 2:
            cp_wA(0).start()
            for c in range(2, NC):
                cp_x(c).start()
            ln_x0(1)
        fold(1, range(g0, g1))
        pk0.append(_nt(_upk(wAT[g0 * 64:g1 * 64, :]), val['xn', 0]))
    val['pk', 0] = jnp.concatenate(pk0, axis=0)

    cp_wA(2).wait()
    prep_wvT()
    m_pk(1)
    v_phik(0)
    m_vT(0)
    v_phik(1)
    m_vT(1)
    m_kv(0)
    m_kv(1)
    cp_wA(0).wait()
    for c in range(2, NC):
        cp_x(c).wait()
    for i in (1, 0, 2):
        cp_wB(i).start()
    cp_woB.start()
    cp_woA.start()
    fold(0)
    ln_x0(2)
    m_pq(0)
    v_phiq(0)
    m_pq(1)
    v_phiq(1)

    def prep_region(c):
        if c == 3:
            cp_wB(1).wait()
            for s in range(8):
                prep_wB(1, s)
        elif c == 4:
            cp_wB(0).wait()
            for s in range(8):
                prep_wB(0, s)
        elif c == 5:
            cp_wB(2).wait()
            for s in range(8):
                prep_wB(2, s)
        elif c == 6:
            cp_woB.wait()
            cp_woA.wait()
            prep_woA()
            for s in range(8):
                prep_woB(s)

    for c in range(2, NC):
        if c + 1 < NC:
            ln_x0(c + 1)
        m_pk(c)
        v_phik(c)
        m_vT(c)
        m_kv(c)
        prep_region(c)
        if c < NC - 1:
            m_pq(c)
            v_phiq(c)
    finalize_kv()

    def b_phase(final):
        m_num(0)
        m_num(1)
        m_pq(NC - 1)
        v_phiq(NC - 1)
        v_o(0)
        for t in range(-1, NC + 2):
            if 2 <= t + 2 < NC:
                m_num(t + 2)
            if 0 <= t + 2 < NC and t + 2 > 0:
                v_o(t + 2)
            if 0 <= t + 1 < NC:
                m_woA(t + 1, final)
                v_ln1(t + 1)
            if 0 <= t < NC:
                m_kB(t)
                m_qB(t)
                v_logits(t)
                m_vB(t)
                v_pv(t)
            if 0 <= t - 1 < NC:
                m_woB(t - 1, final)
                if final:
                    v_out(t - 1)
                else:
                    v_ln2(t - 1)
            if not final and 0 <= t - 2 < NC:
                c = t - 2
                m_pk(c)
                v_phik(c)
                m_vT(c)
                if c < NC - 1:
                    m_pq(c)
                    v_phiq(c)
                m_kv(c)
        if not final:
            finalize_kv()

    b_phase(False)
    b_phase(True)
    for c in range(NC):
        pltpu.make_async_copy(ostage.at[pl.ds(c * C, C), :], out_hbm.at[pl.ds(c * C, C), :], sem_out.at[c]).wait()


@jax.jit
def pallas_interleave_layers__linear_kernel_hedgehog__sliding_local_dilated__prompt_kernel(
    A_x, A_wqkv, A_w_phi, A_wo, B_x, B_wqkv, B_wo,
):
    del B_x
    x = A_x.reshape(S, D)
    wphi = A_w_phi.reshape(H * DH, DH)
    any_spec = pl.BlockSpec(memory_space=pl.ANY)
    out = pl.pallas_call(
        _kernel,
        out_shape=jax.ShapeDtypeStruct((S, D), bf16),
        in_specs=[any_spec] * 6,
        out_specs=any_spec,
        scratch_shapes=[
            pltpu.VMEM((H * DH, DH), bf16),
            pltpu.VMEM((3, C, D), f32),
            pltpu.VMEM((S, D), bf16),
            pltpu.VMEM((D, 3 * D), bf16),
            pltpu.VMEM((3 * D // 2, D), u32),
            pltpu.VMEM((D, D), bf16),
            pltpu.VMEM((D // 2, D), u32),
            pltpu.VMEM((D, 3 * D), bf16),
            pltpu.VMEM((D, D), bf16),
            pltpu.VMEM((3 * D // 2, D), u32),
            pltpu.VMEM((D // 2, D), u32),
            pltpu.VMEM((2, DH * (DH + 1), 128), f32),
            pltpu.VMEM((D, S), u32),
            pltpu.VMEM((S, D), f32),
            pltpu.VMEM((16, 80, 128), f32),
            pltpu.VMEM((16, 40, 128), u32),
            pltpu.VMEM((8, HALO + S, 128), f32),
            pltpu.VMEM((8, HALO + S, 128), f32),
            pltpu.VMEM((24, C, 128), f32),
            pltpu.VMEM((24, C, 128), f32),
            pltpu.VMEM((S, D), bf16),
            pltpu.SemaphoreType.DMA((NC + 12,)),
            pltpu.SemaphoreType.DMA((NC,)),
        ],
        compiler_params=pltpu.CompilerParams(vmem_limit_bytes=124 * 1024 * 1024),
        name="hedgehog_sliding_fused",
    )(x, A_wqkv, wphi, A_wo, B_wqkv, B_wo)
    return out.reshape(1, S, D)
```

```python
import math

import jax
import jax.numpy as jnp
import numpy as np
from jax.experimental import pallas as pl
from jax.experimental.pallas import tpu as pltpu

f32 = jnp.float32
bf16 = jnp.bfloat16
u32 = jnp.uint32

S = 2048
D = 1024
H = 32
DH = 32
C = 256
NC = S // C
LOG2E = math.log2(math.e)
HALO = 16
RB = 32


def _nt(a, b):
    return jax.lax.dot_general(a, b, (((1,), (1,)), ((), ())), preferred_element_type=f32)


def _nn(a, b):
    return jnp.dot(a, b, preferred_element_type=f32)


def _pk(x):
    return pltpu.bitcast(x, u32)


def _upk(x):
    return pltpu.bitcast(x, bf16)


def _rcp(d):
    r = pl.reciprocal(d, approx=True)
    return r * (2.0 - d * r)


def _layernorm(x):
    m = jnp.mean(x, axis=-1, keepdims=True)
    xc = x - m
    v = jnp.mean(xc * xc, axis=-1, keepdims=True)
    return (xc * jax.lax.rsqrt(v + 1e-5)).astype(bf16)


def _layernorm_ref(load):
    m = jnp.mean(load(), axis=-1, keepdims=True)
    xc = load() - m
    r = jax.lax.rsqrt(jnp.mean(xc * xc, axis=-1, keepdims=True) + 1e-5)
    return (load() * r - m * r).astype(bf16)


def _feature_map(p):
    t = p.shape[1]
    p3 = p.reshape(H, DH, t)
    mx = jnp.max(p3, axis=1, keepdims=True)
    mn = jnp.min(p3, axis=1, keepdims=True)
    ep = jnp.exp2(p3 - mx)
    en = jnp.exp2(mn - p3)
    rp = _rcp(jnp.sum(ep, axis=1, keepdims=True))
    rn = _rcp(jnp.sum(en, axis=1, keepdims=True))
    phi = jnp.concatenate([ep * rp, en * rn], axis=1)
    return phi.reshape(2 * D, t)


def _kernel(x_hbm, wA_hbm, wphi_hbm, woA_hbm, wB_hbm, woB_hbm, out_hbm,
            wphi_ref, x1s, xs, wA, wAT, woAs, woA, wB, woBs, wBT, woB, perm, phiq, xres, kvacc, zacc, kvz,
            kscr, vscr, t0, t1, ostage, sem_in, sem_out):
    def cp_x(c):
        return pltpu.make_async_copy(x_hbm.at[pl.ds(c * C, C), :], xs.at[pl.ds(c * C, C), :], sem_in.at[c])

    def cp_wA(i):
        return pltpu.make_async_copy(wA_hbm.at[:, pl.ds(i * D, D)], wA.at[pl.ds(0, D), pl.ds(i * D, D)], sem_in.at[NC + i])

    def cp_wB(i):
        return pltpu.make_async_copy(wB_hbm.at[:, pl.ds(i * D, D)], wB.at[pl.ds(0, D), pl.ds(i * D, D)], sem_in.at[NC + 6 + i])

    WK = [(0, 2), (2, 5), (5, 8)]

    def cp_wk(part):
        g0, g1 = WK[part]
        cols = pl.ds(D + g0 * 128, (g1 - g0) * 128)
        return pltpu.make_async_copy(wA_hbm.at[:, cols], wA.at[pl.ds(0, D), cols], sem_in.at[NC + 9 + part])

    cp_wphi = pltpu.make_async_copy(wphi_hbm, wphi_ref, sem_in.at[NC + 3])
    cp_woA = pltpu.make_async_copy(woA_hbm, woAs.at[pl.ds(0, D), :], sem_in.at[NC + 4])
    cp_woB = pltpu.make_async_copy(woB_hbm, woBs.at[pl.ds(0, D), :], sem_in.at[NC + 5])

    def bd_phi_t(g):
        wp = wphi_ref[g * 128:(g + 1) * 128, :].astype(f32)
        wt = jnp.concatenate([wp] * 4, axis=1)
        r = jax.lax.broadcasted_iota(jnp.int32, (128, 128), 0) // DH
        cc = jax.lax.broadcasted_iota(jnp.int32, (128, 128), 1) // DH
        return jnp.where(r == cc, wt, 0.0).T.astype(bf16)

    def fold(i, groups=range(8)):
        dst = 0 if i == 1 else D
        for g in groups:
            r = _nt(bd[g], wA[0:D, i * D + g * 128: i * D + (g + 1) * 128])
            wAT[dst + g * 64: dst + (g + 1) * 64, :] = _pk((r * LOG2E).astype(bf16))

    def prep_wvT():
        wAT[512:1024, :] = _pk(wA[0:D, 2 * D:3 * D].T)

    def permute_store(val, dst_ref, row0, col0):
        b = (col0 // 128) % perm.shape[0]
        for h in range(H):
            perm[b, pl.ds(h, DH, stride=DH + 1), :] = val[h * DH:(h + 1) * DH, :]
        rows = [perm[b, (DH + 1) * r:(DH + 1) * r + DH, :] for r in range(DH)]
        dst_ref[row0:row0 + 512, col0:col0 + 128] = _pk(jnp.concatenate(rows, axis=0).astype(bf16))

    def prep_wB(i, s):
        w = wB[s * 128:(s + 1) * 128, i * D:(i + 1) * D].astype(f32).T
        permute_store(w, wBT, i * 512, s * 128)

    def prep_woB(s):
        permute_store(woBs[0:D, s * 128:(s + 1) * 128].astype(f32), woB, 0, s * 128)

    def prep_woA():
        woA[...] = _pk(woAs[0:D, :])

    val = {}

    def ln_x0(c):
        val['xn', c] = _layernorm(xs[c * C:(c + 1) * C, :].astype(f32))

    def m_pk(c):
        val['pk', c] = _nt(_upk(wAT[0:512, :]), val['xn', c])

    def m_vT(c):
        val['vT', c] = _nt(_upk(wAT[512:1024, :]), val['xn', c]).astype(bf16)

    def m_pq(c):
        val['pq', c] = _nt(_upk(wAT[1024:1536, :]), val['xn', c])

    def v_phik(c):
        phi = _feature_map(val.pop(('pk', c)))
        zs = phi[:, 0:128] + phi[:, 128:256]
        if c == 0:
            zacc[...] = zs
        else:
            zacc[...] += zs
        val['phik', c] = phi.astype(bf16)

    def v_phiq(c):
        phiq[:, c * C:(c + 1) * C] = _pk(_feature_map(val.pop(('pq', c))).astype(bf16))

    def m_kv(c):
        phik = val.pop(('phik', c))
        vt = val.pop(('vT', c))
        for hp in range(16):
            r = _nt(vt[hp * 64:(hp + 1) * 64, :], phik[hp * 128:(hp + 1) * 128, :])
            if c == 0:
                kvacc[hp] = r
            else:
                kvacc[hp] += r

    def finalize_kv():
        row = jax.lax.broadcasted_iota(jnp.int32, (80, 128), 0)
        head = jnp.where(row < 16, row // 8, (row - 16) // DH)
        keep = head == jax.lax.broadcasted_iota(jnp.int32, (80, 128), 1) // 64
        for hp in range(16):
            z = jnp.sum(zacc[hp * 128:(hp + 1) * 128, :].T, axis=0, keepdims=True)
            full = jnp.concatenate([jnp.broadcast_to(z, (16, 128)), kvacc[hp]], axis=0)
            kvz[hp] = _pk(jnp.where(keep, full, 0.0).astype(bf16))

    def m_num(c):
        val['num', c] = [_nn(_upk(kvz[hp]), _upk(phiq[hp * 64:(hp + 1) * 64, c * C:(c + 1) * C]))
                         for hp in range(16)]

    def v_o(c):
        nums = val.pop(('num', c))
        outs = []
        for hp in range(16):
            num = nums[hp][16:80, :].reshape(2, DH, C)
            den = nums[hp][0:16, :].reshape(2, 8, C) + 1e-6
            r = _rcp(den)
            r = jnp.concatenate([r] * 4, axis=1)
            outs.append((num * r).reshape(64, C).astype(bf16))
        val['o', c] = jnp.concatenate(outs, axis=0).T

    def m_woA(c, final):
        x = xres[c * C:(c + 1) * C, :] if final else xs[c * C:(c + 1) * C, :].astype(f32)
        x1s[c % 3] = x + _nn(val.pop(('o', c)), _upk(woA[...]))

    def v_ln1(c):
        val['xn1', c] = _layernorm_ref(lambda: x1s[c % 3])

    def m_kB(c):
        k = _nt(val['xn1', c], _upk(wBT[512:1024, :]))
        for j in range(8):
            kscr[j, HALO + c * C: HALO + (c + 1) * C, :] = k[:, j * 128:(j + 1) * 128]

    def m_qB(c):
        t = t0 if c % 2 == 0 else t1
        q = _nt(val['xn1', c], _upk(wBT[0:512, :])) * (DH ** -0.5 * LOG2E)
        for j in range(8):
            t[j] = q[:, j * 128:(j + 1) * 128]

    def m_vB(c):
        v = _nt(val.pop(('xn1', c)), _upk(wBT[1024:1536, :]))
        for j in range(8):
            vscr[j, HALO + c * C: HALO + (c + 1) * C, :] = v[:, j * 128:(j + 1) * 128]

    def v_logits(c):
        t = t0 if c % 2 == 0 else t1
        base = HALO + c * C
        for r0 in range(0, C, RB):
            rr = r0
            row = jax.lax.broadcasted_iota(jnp.int32, (RB, 128), 0) + r0
            qs = [t[j, pl.ds(rr, RB), :] for j in range(8)]
            lg = []
            for w in range(8):
                acc = None
                for j in range(8):
                    p = qs[j] * kscr[j, base + r0 - 2 * w: base + r0 - 2 * w + RB, :]
                    acc = p if acc is None else acc + p
                acc = (acc + pltpu.roll(acc, 64, 1)) + (pltpu.roll(acc, 32, 1) + pltpu.roll(acc, 96, 1))
                if c == 0 and w > 0 and r0 < 16:
                    acc = jnp.where(row >= 2 * w, acc, -1e9 * LOG2E)
                lg.append(acc)
            m = lg[0]
            for w in range(1, 8):
                m = jnp.maximum(m, lg[w])
            e = [jnp.exp2(l - m) for l in lg]
            s = e[0]
            for w in range(1, 8):
                s = s + e[w]
            r = _rcp(s)
            for w in range(8):
                t[8 + w, r0:r0 + RB, :] = e[w] * r

    def v_pv(c):
        t = t0 if c % 2 == 0 else t1
        base = HALO + c * C
        for r0 in range(0, C, RB):
            rr = r0
            a = [t[8 + w, pl.ds(rr, RB), :] for w in range(8)]
            for j in range(8):
                acc = None
                for w in range(8):
                    p = a[w] * vscr[j, base + r0 - 2 * w: base + r0 - 2 * w + RB, :]
                    acc = p if acc is None else acc + p
                t[16 + j, r0 // 2:(r0 + RB) // 2, :] = pltpu.bitcast(acc.astype(bf16), f32)

    def m_woB(c, final):
        t = t0 if c % 2 == 0 else t1
        at = jnp.concatenate([_upk(t[16 + j, 0:C // 2, :]) for j in range(8)], axis=1)
        x2 = x1s[c % 3] + _nn(at, _upk(woB[...]))
        if final:
            val['x2', c] = x2
        else:
            xres[c * C:(c + 1) * C, :] = x2

    def v_ln2(c):
        val['xn', c] = _layernorm_ref(lambda: xres[c * C:(c + 1) * C, :])

    def v_out(c):
        ostage[c * C:(c + 1) * C, :] = val.pop(('x2', c)).astype(bf16)
        pltpu.make_async_copy(ostage.at[pl.ds(c * C, C), :], out_hbm.at[pl.ds(c * C, C), :], sem_out.at[c]).start()

    cp_wphi.start()
    cp_x(0).start()
    cp_wk(0).start()
    cp_wk(1).start()
    kscr[:, 0:HALO, :] = jnp.zeros((8, HALO, 128), f32)
    vscr[:, 0:HALO, :] = jnp.zeros((8, HALO, 128), f32)
    cp_wphi.wait()
    cp_x(0).wait()
    bd = [bd_phi_t(g) for g in range(8)]
    ln_x0(0)
    pk0 = []
    for part in range(3):
        g0, g1 = WK[part]
        cp_wk(part).wait()
        if part == 0:
            cp_wk(2).start()
            cp_x(1).start()
        if part == 1:
            cp_x(1).wait()
            cp_wA(2).start()
        if part == 2:
            cp_wA(0).start()
            for c in range(2, NC):
                cp_x(c).start()
            ln_x0(1)
        fold(1, range(g0, g1))
        pk0.append(_nt(_upk(wAT[g0 * 64:g1 * 64, :]), val['xn', 0]))
    val['pk', 0] = jnp.concatenate(pk0, axis=0)

    cp_wA(2).wait()
    prep_wvT()
    m_pk(1)
    v_phik(0)
    m_vT(0)
    v_phik(1)
    m_vT(1)
    m_kv(0)
    m_kv(1)
    cp_wA(0).wait()
    for c in range(2, NC):
        cp_x(c).wait()
    for i in (1, 0, 2):
        cp_wB(i).start()
    cp_woB.start()
    cp_woA.start()
    fold(0)
    ln_x0(2)
    m_pq(0)
    v_phiq(0)
    m_pq(1)
    v_phiq(1)

    def prep_region(c):
        if c == 3:
            cp_wB(1).wait()
            for s in range(8):
                prep_wB(1, s)
        elif c == 4:
            cp_wB(0).wait()
            for s in range(8):
                prep_wB(0, s)
        elif c == 5:
            cp_wB(2).wait()
            for s in range(8):
                prep_wB(2, s)
        elif c == 6:
            cp_woB.wait()
            cp_woA.wait()
            prep_woA()
            for s in range(8):
                prep_woB(s)

    for c in range(2, NC):
        if c + 1 < NC:
            ln_x0(c + 1)
        m_pk(c)
        v_phik(c)
        m_vT(c)
        m_kv(c)
        prep_region(c)
        if c < NC - 1:
            m_pq(c)
            v_phiq(c)
    finalize_kv()

    def b_phase(final):
        m_num(0)
        m_num(1)
        m_pq(NC - 1)
        v_phiq(NC - 1)
        v_o(0)
        for t in range(-1, NC + 2):
            if 2 <= t + 2 < NC:
                m_num(t + 2)
            if 0 <= t + 2 < NC and t + 2 > 0:
                v_o(t + 2)
            if 0 <= t + 1 < NC:
                m_woA(t + 1, final)
                v_ln1(t + 1)
            if 0 <= t < NC:
                m_kB(t)
                m_qB(t)
                v_logits(t)
                m_vB(t)
                v_pv(t)
            if 0 <= t - 1 < NC:
                m_woB(t - 1, final)
                if final:
                    v_out(t - 1)
                else:
                    v_ln2(t - 1)
            if not final and 0 <= t - 2 < NC:
                c = t - 2
                m_pk(c)
                v_phik(c)
                m_vT(c)
                if c < NC - 1:
                    m_pq(c)
                    v_phiq(c)
                m_kv(c)
        if not final:
            finalize_kv()

    b_phase(False)
    b_phase(True)
    for c in range(NC):
        pltpu.make_async_copy(ostage.at[pl.ds(c * C, C), :], out_hbm.at[pl.ds(c * C, C), :], sem_out.at[c]).wait()


@jax.jit
def pallas_interleave_layers__linear_kernel_hedgehog__sliding_local_dilated__prompt_kernel(
    A_x, A_wqkv, A_w_phi, A_wo, B_x, B_wqkv, B_wo,
):
    del B_x
    x = A_x.reshape(S, D)
    wphi = A_w_phi.reshape(H * DH, DH)
    any_spec = pl.BlockSpec(memory_space=pl.ANY)
    out = pl.pallas_call(
        _kernel,
        out_shape=jax.ShapeDtypeStruct((S, D), bf16),
        in_specs=[any_spec] * 6,
        out_specs=any_spec,
        scratch_shapes=[
            pltpu.VMEM((H * DH, DH), bf16),
            pltpu.VMEM((3, C, D), f32),
            pltpu.VMEM((S, D), bf16),
            pltpu.VMEM((D, 3 * D), bf16),
            pltpu.VMEM((3 * D // 2, D), u32),
            pltpu.VMEM((D, D), bf16),
            pltpu.VMEM((D // 2, D), u32),
            pltpu.VMEM((D, 3 * D), bf16),
            pltpu.VMEM((D, D), bf16),
            pltpu.VMEM((3 * D // 2, D), u32),
            pltpu.VMEM((D // 2, D), u32),
            pltpu.VMEM((2, DH * (DH + 1), 128), f32),
            pltpu.VMEM((D, S), u32),
            pltpu.VMEM((S, D), f32),
            pltpu.VMEM((16, 64, 128), f32),
            pltpu.VMEM((2 * D, 128), f32),
            pltpu.VMEM((16, 40, 128), u32),
            pltpu.VMEM((8, HALO + S, 128), f32),
            pltpu.VMEM((8, HALO + S, 128), f32),
            pltpu.VMEM((24, C, 128), f32),
            pltpu.VMEM((24, C, 128), f32),
            pltpu.VMEM((S, D), bf16),
            pltpu.SemaphoreType.DMA((NC + 12,)),
            pltpu.SemaphoreType.DMA((NC,)),
        ],
        compiler_params=pltpu.CompilerParams(vmem_limit_bytes=124 * 1024 * 1024),
        name="hedgehog_sliding_fused",
    )(x, A_wqkv, wphi, A_wo, B_wqkv, B_wo)
    return out.reshape(1, S, D)
```
